```python
import os as _os
_os.environ.setdefault("JAX_PLATFORMS", "cpu")
import jax
import jax.numpy as jnp

def _softmax(x, axis=-1):
    return jax.nn.softmax(x, axis=axis)
def _gelu(x):
    return jax.nn.gelu(x, approximate=True)
def _silu(x):
    return jax.nn.silu(x)
def _sigmoid(x):
    return jax.nn.sigmoid(x)
def _layernorm(x, axis=-1, eps=1e-5):
    m = jnp.mean(x, axis=axis, keepdims=True)
    v = jnp.var(x, axis=axis, keepdims=True)
    return (x - m) / jnp.sqrt(v + eps)
def _scatter_add(tgt, idx, src, axis=0):
    return tgt.at[idx].add(src)
def _segment_sum(src, seg, n):
    return jax.ops.segment_sum(src, seg, n)
class _Rng:
    def __init__(self, key):
        self._k = key
    def _next(self):
        self._k, sub = jax.random.split(self._k)
        return sub
    def normal(self, shape):
        return jax.random.normal(self._next(), shape, dtype=jnp.bfloat16)
    def randint(self, lo, hi, shape):
        return jax.random.randint(self._next(), shape, lo, hi, dtype=jnp.int32)
    def uniform(self, shape, lo=0.0, hi=1.0):
        return jax.random.uniform(self._next(), shape, jnp.bfloat16, lo, hi)
    def permutation(self, n):
        return jax.random.permutation(self._next(), n)


kernel_name = 'sequential_preLN__compressed_kv_cla__dense_activation_mish__decode'

def setup_inputs():
    _rng = _Rng(jax.random.key(int.from_bytes(__import__("os").urandom(4), "little")))
    _w = (lambda a: (lambda t: t.astype(jnp.bfloat16) if jnp.issubdtype(t.dtype, jnp.floating) else t)(jnp.asarray(a)))
    def _A_setup():
        B, H, Sq, Sk, D, M = 1, 32, 1, 8192, 128, 512
        Dc = 4 * D
        return {
            "x": _w((lambda *s: _rng.normal(s) * 0.05)(B, Sq, M)),
            "c_kv": _w((lambda *s: _rng.normal(s) * 0.8)(B, Sk, Dc)),
            "w_q": _w((lambda *s: _rng.normal(s) * 0.8)(M, H, D) * (M ** -0.5)),
            "w_uk": _w((lambda *s: _rng.normal(s) * 0.8)(Dc, H, D) * (Dc ** -0.5)),
            "w_uv": _w((lambda *s: _rng.normal(s) * 0.8)(Dc, H, D) * (Dc ** -0.5)),
            "w_o": _w((lambda *s: _rng.normal(s) * 0.8)(H, D, M) * ((H * D) ** -0.5)),
        }
    _A_in = _A_setup()

    def _B_setup():
        B, S, D, F = 1, 1, 512, 1376
        return {
            "x": _w((lambda *s: _rng.normal(s) * 0.05)(B, S, D)),
            "w1": _w((lambda *s: _rng.normal(s) * 0.2)(D, F) * (D ** -0.5)),
            "b1": _w((lambda *s: _rng.normal(s) * 0.05)(F)),
            "w2": _w((lambda *s: _rng.normal(s) * 0.05)(F, D) * (F ** -0.5)),
        }
    _B_in = _B_setup()

    return {
        "A_x": _A_in["x"],
        "A_c_kv": _A_in["c_kv"],
        "A_w_q": _A_in["w_q"],
        "A_w_uk": _A_in["w_uk"],
        "A_w_uv": _A_in["w_uv"],
        "A_w_o": _A_in["w_o"],
        "B_x": _B_in["x"],
        "B_w1": _B_in["w1"],
        "B_b1": _B_in["b1"],
        "B_w2": _B_in["w2"],
    }

def reference(A_x, A_c_kv, A_w_q, A_w_uk, A_w_uv, A_w_o, B_x, B_w1, B_b1, B_w2):
    def _A_ref(x, c_kv, w_q, w_uk, w_uv, w_o):
        B, Sq, M = x.shape[0], x.shape[1], x.shape[2]
        Sk = c_kv.shape[1]
        H, D = w_q.shape[1], w_q.shape[2]
        q = jnp.einsum("bqm,mhd->bhqd", x, w_q)
        k = jnp.einsum("bkc,chd->bhkd", c_kv, w_uk)
        v = jnp.einsum("bkc,chd->bhkd", c_kv, w_uv)
        scores = jnp.einsum("bhqd,bhkd->bhqk", q, k) * (D ** -0.5)
        off = Sk - Sq
        qi = jnp.arange(Sq)[:, None]
        kj = jnp.arange(Sk)[None, :]
        cmask = kj <= (qi + off)
        scores = jnp.where(cmask[None, None], scores, -1e9)
        p = _softmax(scores, axis=-1)
        ctx = jnp.einsum("bhqk,bhkd->bhqd", p, v)
        return jnp.einsum("bhqd,hdm->bqm", ctx, w_o)

    def _B_ref(x, w1, b1, w2):
        h = jnp.einsum("bsd,df->bsf", x, w1) + b1
        sp = jnp.log1p(jnp.exp(-jnp.abs(h))) + jnp.where(h > 0, h, jnp.zeros_like(h))
        act = h * jnp.tanh(sp)
        return jnp.einsum("bsf,fd->bsd", act, w2)

    x = A_x
    h = x + _A_ref(_layernorm(x, axis=-1), A_c_kv, A_w_q, A_w_uk, A_w_uv, A_w_o)
    h2 = h + _B_ref(_layernorm(h, axis=-1), B_w1, B_b1, B_w2)
    return h2
```

```python
import functools
import jax
import jax.numpy as jnp
import jax.experimental.pallas as pl
import jax.experimental.pallas.tpu as pltpu

F32 = jnp.float32
BF16 = jnp.bfloat16

def _ln(x):
    m = jnp.mean(x, axis=-1, keepdims=True)
    d = x - m
    v = jnp.mean(d * d, axis=-1, keepdims=True)
    return d / jnp.sqrt(v + 1e-5)

def _build(n_kv=4, n_wo=4, f_chunks=(384, 384, 384, 224), G=16):
    H, D, M, Sk, Dc, F = 32, 128, 512, 8192, 512, 1376
    kv_rows = Sk // n_kv
    ho = H // n_wo
    f_off = [0]
    for c in f_chunks:
        f_off.append(f_off[-1] + c)
    assert f_off[-1] == F
    n_f = len(f_chunks)

    def kernel(x_hbm, ckv_hbm, wq_hbm, wuk_hbm, wuv_hbm, wo_hbm, w1t_hbm, b1_hbm, w2_hbm, o_ref,
               x_v, b1_v, wq_v, wuk_v, ckv_v, wuv_v, wo_v, w1_v, w2_v, e_v, r_v, ctx_v, sems):
        cps = {}
        order = []
        def add(name, src, dst):
            i = len(order)
            cps[name] = pltpu.make_async_copy(src, dst, sems.at[i])
            order.append(name)
        add('x', x_hbm, x_v)
        add('wq', wq_hbm, wq_v)
        add('b1', b1_hbm, b1_v)
        add('wuk', wuk_hbm, wuk_v)
        for j in range(n_kv):
            add(('kv', j), ckv_hbm.at[0, pl.ds(j * kv_rows, kv_rows)], ckv_v.at[pl.ds(j * kv_rows, kv_rows)])
        add('wuv', wuv_hbm, wuv_v)
        for j in range(n_wo):
            add(('wo', j), wo_hbm.at[pl.ds(j * ho, ho)], wo_v.at[pl.ds(j * ho, ho)])
        add('w1', w1t_hbm, w1_v)
        for j in range(n_f):
            add(('w2', j), w2_hbm.at[pl.ds(f_off[j], f_chunks[j])], w2_v.at[pl.ds(f_off[j], f_chunks[j])])
        for name in order:
            cps[name].start()

        row = jax.lax.broadcasted_iota(jnp.int32, (H, 128), 0)
        lane = jax.lax.broadcasted_iota(jnp.int32, (H, 128), 1)
        diag = row == (lane % H)

        def wtiles(w_v, t0):
            parts = [w_v[pl.ds(ci * 128 + t0, G)] for ci in range(4)]
            return jnp.stack(parts, axis=1).reshape(G * 128, 128)

        def head_matvec(a, w_v):
            s = jnp.concatenate([a[:, ci * 128:(ci + 1) * 128] for ci in range(4)], axis=0)
            e_v[...] = s.T
            def body(g, acc):
                t0 = pl.multiple_of(g * G, G)
                ls = []
                for i in range(G):
                    r = e_v[pl.ds(t0 + i, 1), :]
                    ls.append(jnp.where(diag, jnp.broadcast_to(r, (H, 128)), 0.0).astype(BF16))
                L = jnp.concatenate(ls, axis=1)
                return acc + jnp.dot(L, wtiles(w_v, t0), preferred_element_type=F32)
            return jax.lax.fori_loop(0, 128 // G, body, jnp.zeros((H, D), F32))

        cps['x'].wait()
        x = x_v[0].astype(F32)
        xn = _ln(x).astype(BF16).astype(F32)
        a1 = jnp.broadcast_to(xn, (H, M))
        cps['wq'].wait()
        q = head_matvec(a1, wq_v).astype(BF16)

        cps['wuk'].wait()
        def body2(g, c):
            t0 = pl.multiple_of(g * G, G)
            o = jax.lax.dot_general(q, wtiles(wuk_v, t0), (((1,), (1,)), ((), ())), preferred_element_type=F32)
            rs = []
            for i in range(G):
                t = jnp.where(diag, o[:, i * 128:(i + 1) * 128], 0.0)
                rs.append(jnp.sum(t, axis=0, keepdims=True))
            r_v[pl.ds(t0, G), :] = jnp.concatenate(rs, axis=0)
            return c
        jax.lax.fori_loop(0, 128 // G, body2, 0)
        rt = r_v[...].T
        qa = jnp.concatenate([rt[ci * 32:(ci + 1) * 32, :] for ci in range(4)], axis=1).astype(BF16)

        m_i = jnp.full((H, 1), -jnp.inf, F32)
        l_i = jnp.zeros((H, 1), F32)
        acc = jnp.zeros((H, Dc), F32)
        for j in range(n_kv):
            cps[('kv', j)].wait()
            kv = ckv_v[pl.ds(j * kv_rows, kv_rows), :]
            s = jax.lax.dot_general(qa, kv, (((1,), (1,)), ((), ())), preferred_element_type=F32) * (D ** -0.5)
            m_new = jnp.maximum(m_i, jnp.max(s, axis=1, keepdims=True))
            alpha = jnp.exp(m_i - m_new)
            p = jnp.exp(s - m_new)
            l_i = alpha * l_i + jnp.sum(p, axis=1, keepdims=True)
            acc = alpha * acc + jnp.dot(p.astype(BF16), kv, preferred_element_type=F32)
            m_i = m_new
        ctx_c = acc / l_i

        cps['wuv'].wait()
        ctx = head_matvec(ctx_c, wuv_v)
        ctx_v[...] = ctx

        out = jnp.zeros((8, M), F32)
        for j in range(n_wo):
            cps[('wo', j)].wait()
            L = jnp.concatenate([jnp.broadcast_to(ctx_v[pl.ds(j * ho + i, 1), :], (8, 128)) for i in range(ho)], axis=1).astype(BF16)
            out = out + jnp.dot(L, wo_v[pl.ds(j * ho, ho)].reshape(ho * 128, M), preferred_element_type=F32)
        h = x + out
        hn = _ln(h).astype(BF16)
        cps['w1'].wait()
        cps['b1'].wait()
        h1 = jax.lax.dot_general(hn, w1_v[...], (((1,), (1,)), ((), ())), preferred_element_type=F32)
        h1 = h1 + b1_v[...].astype(F32).reshape(1, F)
        sp = jnp.log1p(jnp.exp(-jnp.abs(h1))) + jnp.where(h1 > 0, h1, 0.0)
        act = (h1 * jnp.tanh(sp)).astype(BF16)
        y = h
        for j in range(n_f):
            cps[('w2', j)].wait()
            y = y + jnp.dot(act[:, f_off[j]:f_off[j + 1]], w2_v[pl.ds(f_off[j], f_chunks[j]), :], preferred_element_type=F32)
        o_ref[...] = y[0:1, :].astype(o_ref.dtype).reshape(1, 1, M)

    n_sems = 6 + n_kv + n_wo + n_f
    def fn(A_x, A_c_kv, A_w_q, A_w_uk, A_w_uv, A_w_o, B_x, B_w1, B_b1, B_w2):
        return pl.pallas_call(
            kernel,
            out_shape=jax.ShapeDtypeStruct(A_x.shape, A_x.dtype),
            in_specs=[pl.BlockSpec(memory_space=pl.ANY)] * 9,
            out_specs=pl.BlockSpec(memory_space=pltpu.VMEM),
            scratch_shapes=[
                pltpu.VMEM((1, 1, M), BF16), pltpu.VMEM((F,), BF16),
                pltpu.VMEM((M, H, D), BF16), pltpu.VMEM((Dc, H, D), BF16), pltpu.VMEM((Sk, Dc), BF16),
                pltpu.VMEM((Dc, H, D), BF16), pltpu.VMEM((H, D, M), BF16), pltpu.VMEM((F, M), BF16), pltpu.VMEM((F, M), BF16),
                pltpu.VMEM((128, 128), F32), pltpu.VMEM((128, 128), F32), pltpu.VMEM((H, D), F32),
                pltpu.SemaphoreType.DMA((n_sems,)),
            ],
            compiler_params=pltpu.CompilerParams(vmem_limit_bytes=100 * 1024 * 1024),
        )(A_x, A_c_kv, A_w_q, A_w_uk, A_w_uv, A_w_o, B_w1.T, B_b1, B_w2)
    return fn


_kernel_fn = _build()


@jax.jit
def pallas_sequential_preLN__compressed_kv_cla__dense_activation_mish__decode_kernel(
    A_x: jax.Array,
    A_c_kv: jax.Array,
    A_w_q: jax.Array,
    A_w_uk: jax.Array,
    A_w_uv: jax.Array,
    A_w_o: jax.Array,
    B_x: jax.Array,
    B_w1: jax.Array,
    B_b1: jax.Array,
    B_w2: jax.Array,
):
    return _kernel_fn(A_x, A_c_kv, A_w_q, A_w_uk, A_w_uv, A_w_o, B_x, B_w1, B_b1, B_w2)
```

```python
import functools

import jax
import jax.numpy as jnp
import jax.experimental.pallas as pl
import jax.experimental.pallas.tpu as pltpu

F32 = jnp.float32
BF16 = jnp.bfloat16

_G = 16
_KV_SUB = 2048
_F_CHUNKS = (896, 352, 128)
_ROWS = 8
_NT = (((1,), (1,)), ((), ()))


def _layernorm(x):
    m = jnp.mean(x, axis=-1, keepdims=True)
    d = x - m
    v = jnp.mean(d * d, axis=-1, keepdims=True)
    return d / jnp.sqrt(v + 1e-5)


def _body(x_hbm, ckv_hbm, wq_hbm, wuk_hbm, wuv_hbm, wo_hbm, w1t_hbm, b1_hbm, w2_hbm,
          x_v, b1_v, wq_v, wuk_v, ckv_v, wuv_v, wo_v, w1_v, w2_v, e_v, r_v, ctx_v, o_v,
          out_copy, sems):
    Dc, H, D = wuk_v.shape
    Sk = ckv_v.shape[0]
    F, M = w2_v.shape
    NS = 128 // H
    NT = Dc // NS
    f_off = [0]
    for c in _F_CHUNKS:
        f_off.append(f_off[-1] + c)

    plan = [("wq", wq_hbm, wq_v, 1), ("x", x_hbm, x_v, 0), ("wuk", wuk_hbm, wuk_v, 1),
            ("kv", ckv_hbm.at[0], ckv_v, 1), ("wuv", wuv_hbm, wuv_v, 1),
            ("wo", wo_hbm, wo_v, 1), ("w1", w1t_hbm, w1_v, 1), ("b1", b1_hbm, b1_v, 0)]
    for j, c in enumerate(_F_CHUNKS):
        rows = pl.ds(f_off[j], c)
        plan.append((("w2", j), w2_hbm.at[rows], w2_v.at[rows], 1))
    cps = {}
    for i, (name, src, dst, prio) in enumerate(plan):
        cps[name] = pltpu.make_async_copy(src, dst, sems.at[i])
        cps[name].start(priority=prio)

    row = jax.lax.broadcasted_iota(jnp.int32, (H, 128), 0)
    lane = jax.lax.broadcasted_iota(jnp.int32, (H, 128), 1)
    diag = row == (lane % H)

    def wtiles(w_v, t0):
        parts = [w_v[pl.ds(s * NT + t0, _G)] for s in range(NS)]
        return jnp.stack(parts, axis=1).reshape(_G * 128, D)

    def head_matvec(a, w_v, name):
        st = jnp.concatenate([a[:, s * NT:(s + 1) * NT] for s in range(NS)], axis=0)
        e_v[...] = st.T
        cps[name].wait()
        acc = jnp.zeros((H, D), F32)
        for t0 in range(0, NT, _G):
            ls = []
            for i in range(_G):
                r = jnp.broadcast_to(e_v[pl.ds(t0 + i, 1), :], (H, 128))
                ls.append(jnp.where(diag, r, 0.0).astype(BF16))
            acc = acc + jnp.dot(jnp.concatenate(ls, axis=1), wtiles(w_v, t0),
                                preferred_element_type=F32)
        return acc

    cps["x"].wait()
    x = x_v[0].astype(F32)
    xn = _layernorm(x).astype(BF16).astype(F32)
    q = head_matvec(jnp.broadcast_to(xn, (H, M)), wq_v, "wq").astype(BF16)

    cps["wuk"].wait()
    for t0 in range(0, NT, _G):
        o = jax.lax.dot_general(q, wtiles(wuk_v, t0), _NT, preferred_element_type=F32)
        rs = []
        for i in range(_G):
            t = jnp.where(diag, o[:, i * 128:(i + 1) * 128], 0.0)
            rs.append(jnp.sum(t, axis=0, keepdims=True))
        r_v[pl.ds(t0, _G), :] = jnp.concatenate(rs, axis=0)
    rt = r_v[...].T
    qa = jnp.concatenate([rt[s * H:(s + 1) * H, :] for s in range(NS)], axis=1).astype(BF16)

    cps["kv"].wait()
    m_i = l_i = acc = None
    for s0 in range(0, Sk, _KV_SUB):
        kv = ckv_v[pl.ds(s0, _KV_SUB), :]
        s = jax.lax.dot_general(qa, kv, _NT, preferred_element_type=F32) * (D ** -0.5)
        m_blk = jnp.max(s, axis=1, keepdims=True)
        m_new = m_blk if m_i is None else jnp.maximum(m_i, m_blk)
        p = jnp.exp(s - m_new)
        l_blk = jnp.sum(p, axis=1, keepdims=True)
        pv = jnp.dot(p.astype(BF16), kv, preferred_element_type=F32)
        if m_i is None:
            l_i, acc = l_blk, pv
        else:
            alpha = jnp.exp(m_i - m_new)
            l_i = alpha * l_i + l_blk
            acc = alpha * acc + pv
        m_i = m_new
    ctx_c = acc / l_i

    ctx_v[...] = head_matvec(ctx_c, wuv_v, "wuv")
    cps["wo"].wait()
    L = jnp.concatenate(
        [jnp.broadcast_to(ctx_v[pl.ds(h, 1), :], (_ROWS, D)) for h in range(H)], axis=1)
    h = x + jnp.dot(L.astype(BF16), wo_v[...].reshape(H * D, M), preferred_element_type=F32)

    hn = _layernorm(h).astype(BF16)
    cps["w1"].wait()
    cps["b1"].wait()
    h1 = jax.lax.dot_general(hn, w1_v[...], _NT, preferred_element_type=F32)
    h1 = h1 + b1_v[...].astype(F32).reshape(1, F)
    sp = jnp.log1p(jnp.exp(-jnp.abs(h1))) + jnp.where(h1 > 0, h1, 0.0)
    act = (h1 * jnp.tanh(sp)).astype(BF16)

    last = len(_F_CHUNKS) - 1
    a_last = act[0:1, f_off[last]:f_off[last + 1]].astype(F32)
    a_col = jnp.broadcast_to(a_last, (128, 128)).T
    y = h
    for j in range(last):
        cps[("w2", j)].wait()
        y = y + jnp.dot(act[:, f_off[j]:f_off[j + 1]], w2_v[pl.ds(f_off[j], _F_CHUNKS[j]), :],
                        preferred_element_type=F32)
    cps[("w2", last)].wait()
    wl = w2_v[pl.ds(f_off[last], _F_CHUNKS[last]), :].astype(F32)
    parts = [jnp.sum(wl[:, n * 128:(n + 1) * 128] * a_col, axis=0, keepdims=True)
             for n in range(M // 128)]
    y = y[0:1, :] + jnp.concatenate(parts, axis=1)

    o_v[...] = y.astype(o_v.dtype).reshape(1, 1, M)
    out_copy.start()


def _kernel(*refs):
    ins, o_hbm, scratch, out_sem = refs[:9], refs[9], refs[10:-1], refs[-1]
    out_copy = pltpu.make_async_copy(scratch[-1], o_hbm, out_sem.at[0])
    pl.run_scoped(functools.partial(_body, *ins, *scratch, out_copy),
                  pltpu.SemaphoreType.DMA((8 + len(_F_CHUNKS),)))
    out_copy.wait()


@jax.jit
def pallas_sequential_preLN__compressed_kv_cla__dense_activation_mish__decode_kernel(
    A_x: jax.Array,
    A_c_kv: jax.Array,
    A_w_q: jax.Array,
    A_w_uk: jax.Array,
    A_w_uv: jax.Array,
    A_w_o: jax.Array,
    B_x: jax.Array,
    B_w1: jax.Array,
    B_b1: jax.Array,
    B_w2: jax.Array,
):
    M = A_x.shape[-1]
    _, Sk, Dc = A_c_kv.shape
    _, H, D = A_w_q.shape
    F = B_b1.shape[0]
    dt = A_x.dtype
    return pl.pallas_call(
        _kernel,
        out_shape=jax.ShapeDtypeStruct(A_x.shape, dt),
        in_specs=[pl.BlockSpec(memory_space=pl.ANY)] * 9,
        out_specs=pl.BlockSpec(memory_space=pl.ANY),
        scratch_shapes=[
            pltpu.VMEM((1, 1, M), dt), pltpu.VMEM((F,), dt),
            pltpu.VMEM((M, H, D), dt), pltpu.VMEM((Dc, H, D), dt), pltpu.VMEM((Sk, Dc), dt),
            pltpu.VMEM((Dc, H, D), dt), pltpu.VMEM((H, D, M), dt),
            pltpu.VMEM((F, M), dt), pltpu.VMEM((F, M), dt),
            pltpu.VMEM((128, 128), F32), pltpu.VMEM((128, 128), F32), pltpu.VMEM((H, D), F32),
            pltpu.VMEM((1, 1, M), dt),
            pltpu.SemaphoreType.DMA((1,)),
        ],
        compiler_params=pltpu.CompilerParams(vmem_limit_bytes=100 * 1024 * 1024),
    )(A_x, A_c_kv, A_w_q, A_w_uk, A_w_uv, A_w_o, B_w1.T, B_b1, B_w2)
```
